```python
import os as _os
_os.environ.setdefault("JAX_PLATFORMS", "cpu")
import jax
import jax.numpy as jnp

def _softmax(x, axis=-1):
    return jax.nn.softmax(x, axis=axis)
def _gelu(x):
    return jax.nn.gelu(x, approximate=True)
def _silu(x):
    return jax.nn.silu(x)
def _sigmoid(x):
    return jax.nn.sigmoid(x)
def _layernorm(x, axis=-1, eps=1e-5):
    m = jnp.mean(x, axis=axis, keepdims=True)
    v = jnp.var(x, axis=axis, keepdims=True)
    return (x - m) / jnp.sqrt(v + eps)
def _scatter_add(tgt, idx, src, axis=0):
    return tgt.at[idx].add(src)
def _segment_sum(src, seg, n):
    return jax.ops.segment_sum(src, seg, n)
class _Rng:
    def __init__(self, key):
        self._k = key
    def _next(self):
        self._k, sub = jax.random.split(self._k)
        return sub
    def normal(self, shape):
        return jax.random.normal(self._next(), shape, dtype=jnp.bfloat16)
    def randint(self, lo, hi, shape):
        return jax.random.randint(self._next(), shape, lo, hi, dtype=jnp.int32)
    def uniform(self, shape, lo=0.0, hi=1.0):
        return jax.random.uniform(self._next(), shape, jnp.bfloat16, lo, hi)
    def permutation(self, n):
        return jax.random.permutation(self._next(), n)


kernel_name = 'gated_mix__compressed_kv_cla__linear_attn_block__prompt'

def setup_inputs():
    _rng = _Rng(jax.random.key(int.from_bytes(__import__("os").urandom(4), "little")))
    _w = (lambda a: (lambda t: t.astype(jnp.bfloat16) if jnp.issubdtype(t.dtype, jnp.floating) else t)(jnp.asarray(a)))
    def _A_setup():
        B, H, Sq, Sk, D, M = 1, 16, 2048, 2048, 256, 448
        Dc = 4 * D
        return {
            "x": _w((lambda *s: _rng.normal(s) * 0.05)(B, Sq, M)),
            "c_kv": _w((lambda *s: _rng.normal(s) * 0.8)(B, Sk, Dc)),
            "w_q": _w((lambda *s: _rng.normal(s) * 3.2)(M, H, D) * (M ** -0.5)),
            "w_uk": _w((lambda *s: _rng.normal(s) * 3.2)(Dc, H, D) * (Dc ** -0.5)),
            "w_uv": _w((lambda *s: _rng.normal(s) * 0.8)(Dc, H, D) * (Dc ** -0.5)),
            "w_o": _w((lambda *s: _rng.normal(s) * 0.8)(H, D, M) * ((H * D) ** -0.5)),
        }
    _A_in = _A_setup()

    def _B_setup():
        B, S, D = 1, 2048, 448
        return {
            "x": _w((lambda *s: _rng.normal(s) * 0.05)(B, S, D)),
            "wqkv": _w((lambda *s: _rng.normal(s) * 1.6)(D, 3 * D)),
            "wo": _w((lambda *s: _rng.normal(s) * 0.4)(D, D)),
        }
    _B_in = _B_setup()

    return {
        "A_x": _A_in["x"],
        "A_c_kv": _A_in["c_kv"],
        "A_w_q": _A_in["w_q"],
        "A_w_uk": _A_in["w_uk"],
        "A_w_uv": _A_in["w_uv"],
        "A_w_o": _A_in["w_o"],
        "B_x": _B_in["x"],
        "B_wqkv": _B_in["wqkv"],
        "B_wo": _B_in["wo"],
        "gate_w": _w((lambda *s: _rng.normal(s) * 0.05)(448) * 16.0),
    }

def reference(A_x, A_c_kv, A_w_q, A_w_uk, A_w_uv, A_w_o, B_x, B_wqkv, B_wo, gate_w):
    def _A_ref(x, c_kv, w_q, w_uk, w_uv, w_o):
        B, Sq, M = x.shape[0], x.shape[1], x.shape[2]
        Sk = c_kv.shape[1]
        H, D = w_q.shape[1], w_q.shape[2]
        q = jnp.einsum("bqm,mhd->bhqd", x, w_q)
        k = jnp.einsum("bkc,chd->bhkd", c_kv, w_uk)
        v = jnp.einsum("bkc,chd->bhkd", c_kv, w_uv)
        scores = jnp.einsum("bhqd,bhkd->bhqk", q, k) * (D ** -0.5)
        off = Sk - Sq
        qi = jnp.arange(Sq)[:, None]
        kj = jnp.arange(Sk)[None, :]
        cmask = kj <= (qi + off)
        scores = jnp.where(cmask[None, None], scores, -1e9)
        p = _softmax(scores, axis=-1)
        ctx = jnp.einsum("bhqk,bhkd->bhqd", p, v)
        return jnp.einsum("bhqd,hdm->bqm", ctx, w_o)

    def _B_ref(x, wqkv, wo):
        B, S, D = x.shape
        H = 16; Dh = D // H
        qkv = (lambda x, *d: x.transpose(*d))((x @ wqkv).reshape(B, S, 3, H, Dh), 2, 0, 3, 1, 4)
        q, k, v = qkv[0], qkv[1], qkv[2]
        phi = lambda t: jnp.where(t > 0, t + 1, jnp.exp(t)) + 1e-6
        pq, pk = phi(q), phi(k)
        kv = jnp.einsum("bhsd,bhse->bhde", pk, v)
        z = jnp.einsum("bhsd->bhd", pk)
        num = jnp.einsum("bhqd,bhde->bhqe", pq, kv)
        den = jnp.einsum("bhqd,bhd->bhq", pq, z)[..., None] + 1e-6
        o = num / den
        return (lambda x, *d: x.transpose(*d))(o, 0, 2, 1, 3).reshape(B, S, D) @ wo

    x = A_x
    g = _sigmoid((x * gate_w).sum(-1, keepdims=True))
    a = _A_ref(x, A_c_kv, A_w_q, A_w_uk, A_w_uv, A_w_o)
    b = _B_ref(x, B_wqkv, B_wo)
    return g * a + (1 - g) * b
```

```python
import functools

import jax
import jax.numpy as jnp
from jax import lax
import jax.experimental.pallas as pl
import jax.experimental.pallas.tpu as pltpu

S, M, DC, H, D = 2048, 448, 1024, 16, 256
DH = 28
F32, BF16, U32 = jnp.float32, jnp.bfloat16, jnp.uint32
NN = (((1,), (0,)), ((), ()))
NT = (((1,), (1,)), ((), ()))
TN = (((0,), (0,)), ((), ()))
LOG2E = 1.4426950408889634
BQ = 256
CW = 256
CB = 512


def _dot(a, b, dn=NN):
    return lax.dot_general(a, b, dn, preferred_element_type=F32)


def _phi(t):
    return jnp.where(t > 0, t + 1.0, jnp.exp(t)) + 1e-6


def _head_of(idx):
    return (idx * 2341) >> 16


def _kernel(xT_hbm, ckv_hbm, wq_hbm, wuk_hbm, wuv_hbm, woT_hbm, wqkv_hbm, wob_hbm, gw_hbm,
            outT_hbm,
            xT_v, ckv_v, wq0, wq1, wk0, wk1, wv0, wv1, woT_v, wqkv_v, wob_v, gw_v,
            acc, g_s, x_s, q_s, k_s, v_s, c_s, pq_s, gc_s, out_v, kv_s, lhs_s, w2_s, zs_s,
            sems, osem, xsem):
    wq_v, wk_v, wv_v = (wq0, wq1), (wk0, wk1), (wv0, wv1)
    nc = S // CB
    nb = S // BQ
    copies = {}

    def add(name, src, dst):
        copies[name] = pltpu.make_async_copy(src, dst, sems.at[len(copies)])

    add("wqkv", wqkv_hbm, wqkv_v)
    add("gw", gw_hbm, gw_v)
    add("wob", wob_hbm, wob_v)
    for t in range(2):
        add(f"wq{t}", wq_hbm.at[:, pl.ds(t * 128, 128)], wq_v[t].bitcast(BF16))
    add("ckv", ckv_hbm, ckv_v)
    for t in range(2):
        add(f"wk{t}", wuk_hbm.at[:, pl.ds(t * 128, 128)], wk_v[t].bitcast(BF16))
    for t in range(2):
        add(f"wv{t}", wuv_hbm.at[:, pl.ds(t * 128, 128)], wv_v[t].bitcast(BF16))
    add("wo", woT_hbm, woT_v)

    def xcopy(c):
        cs = pl.multiple_of(c * CB, CB)
        return pltpu.make_async_copy(xT_hbm.at[:, pl.ds(cs, CB)], xT_v.at[:, pl.ds(cs, CB)], xsem.at[c])

    copies["wqkv"].start()
    copies["gw"].start()
    xcopy(0).start()
    copies["wqkv"].wait()
    copies["gw"].wait()
    xcopy(0).wait()
    for c in range(1, nc):
        xcopy(c).start()
    copies["wob"].start()

    wT = wqkv_v[...].T
    gw16 = jnp.broadcast_to(gw_v[...], (16, M))
    lhs_s[...] = jnp.concatenate([wT, gw16], axis=0)
    kv_s[...] = jnp.zeros_like(kv_s)
    pieces = [(0, 144, 0, 128), (112, 288, 128, 256), (240, 400, 256, 384), (352, 448, 384, 448)]
    offs = [0, 160, 352, 528, 640]
    ones16 = jnp.ones((16, CB), BF16)

    def b1(c, carry):
        cs = pl.multiple_of(c * CB, CB)

        @pl.when(c > 0)
        def _():
            xcopy(c).wait()

        @pl.when(c == 1)
        def _():
            for n in ("wq0", "wq1", "ckv", "wk0", "wk1", "wv0", "wv1", "wo"):
                copies[n].start()

        xc = xT_v[:, pl.ds(cs, CB)]
        x_s[pl.ds(cs, CB), :] = xc.T
        t = _dot(lhs_s[...], xc)
        pq_s[:, pl.ds(cs, CB)] = _phi(t[0:M])
        pk = _phi(t[M:2 * M]).astype(BF16)
        vb = t[2 * M:3 * M].astype(BF16)
        g8 = jax.nn.sigmoid(t[3 * M:3 * M + 8])
        g_s[:, pl.ds(cs, CB)] = g8
        gc_s[pl.ds(cs, CB), :] = jnp.concatenate([g8] * 16, axis=0).T
        for n, (r0, r1, c0, c1) in enumerate(pieces):
            l_ = jnp.concatenate([vb[r0:r1], ones16], axis=0)
            pkp = pk[c0:c1]
            if c1 - c0 < 128:
                pkp = jnp.concatenate([pkp, jnp.zeros((128 - (c1 - c0), CB), BF16)], axis=0)
            kv_s[offs[n]:offs[n + 1], :] += _dot(l_, pkp, NT)
        return carry

    lax.fori_loop(0, nc, b1, 0)

    cols, zs = [], []
    for n, (r0, r1, c0, c1) in enumerate(pieces):
        w = c1 - c0
        kvt = kv_s[offs[n]:offs[n + 1], 0:w]
        hr = _head_of(lax.broadcasted_iota(jnp.int32, (r1 - r0, w), 0) + r0)
        hc = _head_of(lax.broadcasted_iota(jnp.int32, (r1 - r0, w), 1) + c0)
        parts = []
        if r0 > 0:
            parts.append(jnp.zeros((r0, w), F32))
        parts.append(jnp.where(hr == hc, kvt[0:r1 - r0], 0.0))
        if r1 < M:
            parts.append(jnp.zeros((M - r1, w), F32))
        cols.append(jnp.concatenate(parts, axis=0))
        zs.append(kvt[r1 - r0:r1 - r0 + 8])
    kvT = jnp.concatenate(cols, axis=1).astype(BF16)
    z8 = jnp.concatenate(zs, axis=1)
    copies["wob"].wait()
    w2_s[...] = _dot(wob_v[...], kvT, TN).astype(BF16)
    hi = lax.broadcasted_iota(jnp.int32, (16, M), 0)
    ci = lax.broadcasted_iota(jnp.int32, (16, M), 1)
    zs_s[...] = jnp.where(hi == _head_of(ci), jnp.concatenate([z8, z8], axis=0), 0.0).astype(BF16)
    sub = lax.broadcasted_iota(jnp.int32, (8, CB), 0)

    copies["wq0"].wait()
    copies["wq1"].wait()

    def qproj(j):
        for par in range(2):
            outs = []
            for t in range(2):
                u = wq_v[t][pl.ds(j, M, stride=H // 2), :]
                u = (u << 16) if par == 0 else (u & jnp.uint32(0xFFFF0000))
                outs.append(pltpu.bitcast(u, F32).astype(BF16))
            w = jnp.concatenate(outs, axis=1)
            q_s[2 * j + par] = (_dot(x_s[...], w) * (LOG2E * D ** -0.5)).astype(BF16)

    def b2(c, carry):
        cs = pl.multiple_of(c * CB, CB)
        pq = pq_s[:, pl.ds(cs, CB)]
        den = _dot(zs_s[...], pq.astype(BF16)) + 1e-6
        rden = (1.0 - jnp.concatenate([g_s[:, pl.ds(cs, CB)]] * 2, axis=0)) / den
        rows = []
        for r in range(M // 8):
            ha, hb = (8 * r) // DH, (8 * r + 7) // DH
            ra = jnp.broadcast_to(rden[ha:ha + 1], (8, CB))
            if ha != hb:
                rb = jnp.broadcast_to(rden[hb:hb + 1], (8, CB))
                ra = jnp.where(sub < (hb * DH - 8 * r), ra, rb)
            rows.append(ra)
        pqn = (pq * jnp.concatenate(rows, axis=0)).astype(BF16)
        acc[:, pl.ds(cs, CB)] = _dot(w2_s[...], pqn)
        for u_ in range(H // 2 // nc):
            qproj(c * (H // 2 // nc) + u_)
        return carry

    lax.fori_loop(0, nc, b2, 0)

    for n in ("ckv", "wk0", "wk1", "wv0", "wv1", "wo"):
        copies[n].wait()

    def extract(bufs, h, rows):
        j = h // 2
        sh = (16 * (1 - (h % 2))).astype(U32)
        outs = []
        for t in range(2):
            u = bufs[t][pl.ds(j, rows, stride=H // 2), :]
            u = (u << sh) & jnp.uint32(0xFFFF0000)
            outs.append(pltpu.bitcast(u, F32).astype(BF16))
        return jnp.concatenate(outs, axis=1)

    ocp = [pltpu.make_async_copy(out_v.at[:, pl.ds(i * BQ, BQ)], outT_hbm.at[:, pl.ds(i * BQ, BQ)], osem.at[i])
           for i in range(nb)]
    hb = BQ // 2

    def head(h, carry):
        k_s[...] = _dot(ckv_v[...], extract(wk_v, h, DC)).astype(BF16)
        v_s[...] = _dot(ckv_v[...], extract(wv_v, h, DC)).astype(BF16)
        q_h = q_s.at[h]
        woT = woT_v[h]
        r2 = lax.broadcasted_iota(jnp.int32, (BQ, hb), 0)
        c2 = lax.broadcasted_iota(jnp.int32, (BQ, hb), 1)

        def scores(i):
            q = q_h[i * BQ:(i + 1) * BQ, :]
            L = (i + 1) * BQ
            chunks = []
            for a in range(0, L - BQ, CW):
                b = min(a + CW, L - BQ)
                chunks.append((a, b, _dot(q, k_s[a:b, :], NT)))
            sA = _dot(q, k_s[L - BQ:L - hb, :], NT)
            sA = jnp.where(c2 <= r2, sA, -1e30)
            chunks.append((L - BQ, L - hb, sA))
            sB = _dot(q_h[i * BQ + hb:(i + 1) * BQ, :], k_s[L - hb:L, :], NT)
            sB = jnp.where(c2[:hb] <= r2[:hb], sB, -1e30)
            m = None
            for (_, _, s) in chunks:
                mm = jnp.max(s, axis=1, keepdims=True)
                m = mm if m is None else jnp.maximum(m, mm)
            mB = jnp.maximum(m[hb:], jnp.max(sB, axis=1, keepdims=True))
            m = jnp.concatenate([m[:hb], mB], axis=0)
            return chunks, m, sB

        def pv(i, sc):
            chunks, m, sB = sc
            L = (i + 1) * BQ
            ctx = None
            l = None
            pB = jnp.exp2(sB - m[hb:])
            lB = jnp.sum(pB, axis=1, keepdims=True)
            cB = _dot(pB.astype(BF16), v_s[L - hb:L, :])
            for (a, b, s) in chunks:
                p = jnp.exp2(s - m)
                ll = jnp.sum(p, axis=1, keepdims=True)
                l = ll if l is None else l + ll
                d_ = _dot(p.astype(BF16), v_s[a:b, :])
                ctx = d_ if ctx is None else ctx + d_
            l = jnp.concatenate([l[:hb], l[hb:] + lB], axis=0)
            ctx = jnp.concatenate([ctx[:hb], ctx[hb:] + cB], axis=0)
            rr = gc_s[i * BQ:(i + 1) * BQ, :] / l
            return jnp.concatenate([ctx[:, :128] * rr, ctx[:, 128:] * rr], axis=1).astype(BF16)

        def oproj(i):
            new = acc[:, i * BQ:(i + 1) * BQ] + _dot(woT, c_s[i * BQ:(i + 1) * BQ, :], NT)
            acc[:, i * BQ:(i + 1) * BQ] = new
            out_v[:, i * BQ:(i + 1) * BQ] = new.astype(BF16)

            @pl.when(h == H - 1)
            def _():
                ocp[i].start()

        idx = list(reversed(range(nb)))
        sc = scores(idx[0])
        for n, i in enumerate(idx):
            cur = sc
            if n + 1 < nb:
                sc = scores(idx[n + 1])
            c_s[i * BQ:(i + 1) * BQ, :] = pv(i, cur)
            if n > 0:
                oproj(idx[n - 1])
        oproj(idx[-1])
        return carry

    lax.fori_loop(0, H, head, 0)
    for cp in ocp:
        cp.wait()


@jax.jit
def pallas_gated_mix__compressed_kv_cla__linear_attn_block__prompt_kernel(
    A_x: jax.Array,
    A_c_kv: jax.Array,
    A_w_q: jax.Array,
    A_w_uk: jax.Array,
    A_w_uv: jax.Array,
    A_w_o: jax.Array,
    B_x: jax.Array,
    B_wqkv: jax.Array,
    B_wo: jax.Array,
    gate_w: jax.Array,
):
    del B_x
    xT = jnp.swapaxes(A_x, 1, 2).reshape(M, S)
    ckv = A_c_kv.reshape(S, DC)
    wq = A_w_q.reshape(M * H, D)
    wuk = A_w_uk.reshape(DC * H, D)
    wuv = A_w_uv.reshape(DC * H, D)
    woT = jnp.swapaxes(A_w_o, 1, 2)
    gw = gate_w.reshape(1, M)
    anyspec = pl.BlockSpec(memory_space=pl.ANY)
    outT = pl.pallas_call(
        _kernel,
        out_shape=jax.ShapeDtypeStruct((M, S), BF16),
        in_specs=[anyspec] * 9,
        out_specs=anyspec,
        scratch_shapes=[
            pltpu.VMEM((M, S), BF16), pltpu.VMEM((S, DC), BF16),
            pltpu.VMEM((M * H // 2, 128), U32), pltpu.VMEM((M * H // 2, 128), U32),
            pltpu.VMEM((DC * H // 2, 128), U32), pltpu.VMEM((DC * H // 2, 128), U32),
            pltpu.VMEM((DC * H // 2, 128), U32), pltpu.VMEM((DC * H // 2, 128), U32),
            pltpu.VMEM((H, M, D), BF16), pltpu.VMEM((M, 3 * M), BF16), pltpu.VMEM((M, M), BF16),
            pltpu.VMEM((1, M), BF16),
            pltpu.VMEM((M, S), F32), pltpu.VMEM((8, S), F32),
            pltpu.VMEM((S, M), BF16),
            pltpu.VMEM((H, S, D), BF16), pltpu.VMEM((S, D), BF16), pltpu.VMEM((S, D), BF16),
            pltpu.VMEM((S, D), BF16),
            pltpu.VMEM((M, S), F32),
            pltpu.VMEM((S, 128), F32),
            pltpu.VMEM((M, S), BF16),
            pltpu.VMEM((640, 128), F32), pltpu.VMEM((3 * M + 16, M), BF16), pltpu.VMEM((M, M), BF16),
            pltpu.VMEM((16, M), BF16),
            pltpu.SemaphoreType.DMA((12,)),
            pltpu.SemaphoreType.DMA((S // BQ,)),
            pltpu.SemaphoreType.DMA((S // CB,)),
        ],
        compiler_params=pltpu.CompilerParams(vmem_limit_bytes=100 * 1024 * 1024),
    )(xT, ckv, wq, wuk, wuv, woT, B_wqkv, B_wo, gw)
    return jnp.swapaxes(outT.reshape(1, M, S), 1, 2)
```

```python
import functools

import jax
import jax.numpy as jnp
from jax import lax
import jax.experimental.pallas as pl
import jax.experimental.pallas.tpu as pltpu

S, M, DC, H, D = 2048, 448, 1024, 16, 256
DH = 28
F32, BF16, U32 = jnp.float32, jnp.bfloat16, jnp.uint32
NN = (((1,), (0,)), ((), ()))
NT = (((1,), (1,)), ((), ()))
TN = (((0,), (0,)), ((), ()))
LOG2E = 1.4426950408889634
BQ = 256
CW = 256
CB = 512


def _dot(a, b, dn=NN):
    return lax.dot_general(a, b, dn, preferred_element_type=F32)


def _b16(u):
    return pltpu.bitcast(u, BF16)


def _u32(x):
    return pltpu.bitcast(x.astype(BF16), U32)


def _ld(ref, r0, r1):
    if ref.dtype == U32:
        return _b16(ref[r0 // 2:r1 // 2, :])
    return ref[r0:r1, :]


def _la(ref):
    return _b16(ref[...]) if ref.dtype == U32 else ref[...]


def _cv(ref, x):
    return _u32(x) if ref.dtype == U32 else x.astype(BF16)


def _bf(ref):
    return ref.bitcast(BF16) if ref.dtype == U32 else ref


def _phi(t):
    return jnp.where(t > 0, t + 1.0, jnp.exp(t)) + 1e-6


def _head_of(idx):
    return (idx * 2341) >> 16


def _kernel(xT_hbm, ckv_hbm, wq_hbm, wuk_hbm, wuv_hbm, woT_hbm, wqkv_hbm, wob_hbm, gw_hbm,
            outT_hbm,
            xT_v, ckv_v, wq_v, wk_v, wv_v, woT_v, wqkv_v, wob_v, gw_v,
            acc, g_s, x_s, q_s, k_s, v_s, c_s, pq_s, gc_s, out_v, kv_s, lhs_s, w2_s, zs_s,
            sems, osem, xsem):
    nc = S // CB
    nb = S // BQ
    copies = {}

    def add(name, src, dst):
        copies[name] = pltpu.make_async_copy(src, dst, sems.at[len(copies)])

    add("wqkv", wqkv_hbm.at[:, pl.ds(0, 512)], wqkv_v.at[:, pl.ds(0, 512)])
    add("wqkv2", wqkv_hbm.at[:, pl.ds(512, 3 * M - 512)], wqkv_v.at[:, pl.ds(512, 3 * M - 512)])
    add("gw", gw_hbm, gw_v)
    add("wob", wob_hbm, wob_v)
    for j in range(H // 2):
        add(f"wq{j}", wq_hbm.bitcast(U32).at[:, j, :], wq_v.at[j])
    add("ckv", ckv_hbm, _bf(ckv_v))
    for j in range(H // 2):
        add(f"wk{j}", wuk_hbm.bitcast(U32).at[:, j, :], wk_v.at[j])
        add(f"wv{j}", wuv_hbm.bitcast(U32).at[:, j, :], wv_v.at[j])
    add("wo", woT_hbm, _bf(woT_v))

    def xcopy(c):
        cs = pl.multiple_of(c * CB, CB)
        return pltpu.make_async_copy(xT_hbm.at[:, pl.ds(cs, CB)], _bf(xT_v).at[:, pl.ds(cs, CB)], xsem.at[c])

    copies["wqkv"].start()
    copies["wqkv2"].start()
    copies["gw"].start()
    xcopy(0).start()
    copies["wqkv"].wait()
    for c in range(1, nc):
        xcopy(c).start()
    copies["wob"].start()

    lhs_s[0:256, :] = _cv(lhs_s, wqkv_v[:, 0:512].T)
    copies["wqkv2"].wait()
    copies["gw"].wait()
    wT = wqkv_v[:, 512:].T
    gw16 = jnp.broadcast_to(gw_v[...][None, :], (16, M))
    lhs_s[256:, :] = _cv(lhs_s, jnp.concatenate([wT, gw16], axis=0))
    kv_s[...] = jnp.zeros_like(kv_s)
    pieces = [(0, 144, 0, 128), (112, 288, 128, 256), (240, 400, 256, 384), (352, 448, 384, 448)]
    offs = [0, 160, 352, 528, 640]
    ones16 = jnp.ones((16, CB), BF16)

    def b1(c, carry):
        cs = pl.multiple_of(c * CB, CB)

        xcopy(c).wait()

        @pl.when(c == 1)
        def _():
            for n in copies:
                if n not in ("wqkv", "wqkv2", "gw", "wob"):
                    copies[n].start()

        xc = _la(xT_v.at[:, pl.ds(cs, CB)])
        xr = CB // (2 if x_s.dtype == U32 else 1)
        x_s[pl.ds(pl.multiple_of(c * xr, xr), xr), :] = _cv(x_s, xc.T)
        t = _dot(_la(lhs_s), xc)
        pq_s[:, pl.ds(cs, CB)] = _phi(t[0:M])
        pk = _phi(t[M:2 * M]).astype(BF16)
        vb = t[2 * M:3 * M].astype(BF16)
        g8 = jax.nn.sigmoid(t[3 * M:3 * M + 8])
        g_s[:, pl.ds(cs, CB)] = g8
        gc_s[pl.ds(cs, CB), :] = jnp.concatenate([g8] * 16, axis=0).T
        for n, (r0, r1, c0, c1) in enumerate(pieces):
            l_ = jnp.concatenate([vb[r0:r1], ones16], axis=0)
            pkp = pk[c0:c1]
            if c1 - c0 < 128:
                pkp = jnp.concatenate([pkp, jnp.zeros((128 - (c1 - c0), CB), BF16)], axis=0)
            kv_s[offs[n]:offs[n + 1], :] += _dot(l_, pkp, NT)
        return carry

    lax.fori_loop(0, nc, b1, 0)

    copies["wob"].wait()
    cols, zs = [], []
    for n, (r0, r1, c0, c1) in enumerate(pieces):
        kvt = kv_s[offs[n]:offs[n + 1], :]
        hr = _head_of(lax.broadcasted_iota(jnp.int32, (r1 - r0, 128), 0) + r0)
        hc = _head_of(lax.broadcasted_iota(jnp.int32, (r1 - r0, 128), 1) + c0)
        kvm = jnp.where(hr == hc, kvt[0:r1 - r0], 0.0).astype(BF16)
        cols.append(_dot(wob_v[r0:r1, :], kvm, TN)[:, :c1 - c0])
        zs.append(kvt[r1 - r0:r1 - r0 + 8, :c1 - c0])
    w2_s[...] = _cv(w2_s, jnp.concatenate(cols, axis=1))
    z8 = jnp.concatenate(zs, axis=1)
    hi = lax.broadcasted_iota(jnp.int32, (16, M), 0)
    ci = lax.broadcasted_iota(jnp.int32, (16, M), 1)
    zs_s[...] = jnp.where(hi == _head_of(ci), jnp.concatenate([z8, z8], axis=0), 0.0).astype(BF16)
    sub = lax.broadcasted_iota(jnp.int32, (8, CB), 0)

    with jax.named_scope("waitq"):
        for j in range(H // 2):
            copies[f"wq{j}"].wait()

    def qproj(j):
        for par in range(2):
            u = wq_v[j]
            u = (u << 16) if par == 0 else (u & jnp.uint32(0xFFFF0000))
            w = pltpu.bitcast(u, F32).astype(BF16)
            q_s[2 * j + par] = _cv(q_s, _dot(_la(x_s), w) * (LOG2E * D ** -0.5))

    def b2(c, carry):
        cs = pl.multiple_of(c * CB, CB)
        pq = pq_s[:, pl.ds(cs, CB)]
        den = _dot(zs_s[...], pq.astype(BF16)) + 1e-6
        rden = (1.0 - jnp.concatenate([g_s[:, pl.ds(cs, CB)]] * 2, axis=0)) / den
        rows = []
        for r in range(M // 8):
            ha, hb = (8 * r) // DH, (8 * r + 7) // DH
            ra = jnp.broadcast_to(rden[ha:ha + 1], (8, CB))
            if ha != hb:
                rb = jnp.broadcast_to(rden[hb:hb + 1], (8, CB))
                ra = jnp.where(sub < (hb * DH - 8 * r), ra, rb)
            rows.append(ra)
        pqn = (pq * jnp.concatenate(rows, axis=0)).astype(BF16)
        acc[:, pl.ds(cs, CB)] = _dot(_la(w2_s), pqn)
        for u_ in range(H // 2 // nc):
            qproj(c * (H // 2 // nc) + u_)
        return carry

    lax.fori_loop(0, nc, b2, 0)

    with jax.named_scope("waitkv"):
        for n in copies:
            if n not in ("wqkv", "wqkv2", "gw", "wob") and not n.startswith("wq"):
                copies[n].wait()

    def extract(buf, h):
        sh = (16 * (1 - (h % 2))).astype(U32)
        u = (buf[h // 2] << sh) & jnp.uint32(0xFFFF0000)
        return pltpu.bitcast(u, F32).astype(BF16)

    ocp = [pltpu.make_async_copy(_bf(out_v).at[:, pl.ds(i * BQ, BQ)], outT_hbm.at[:, pl.ds(i * BQ, BQ)], osem.at[i])
           for i in range(nb)]
    hb = BQ // 2

    def head(h, carry):
        k_s[...] = _cv(k_s, _dot(_la(ckv_v), extract(wk_v, h)))
        v_s[...] = _cv(v_s, _dot(_la(ckv_v), extract(wv_v, h)))
        q_h = q_s.at[h]
        woT = _la(woT_v.at[h])
        r2 = lax.broadcasted_iota(jnp.int32, (BQ, hb), 0)
        c2 = lax.broadcasted_iota(jnp.int32, (BQ, hb), 1)

        def scores(i):
            q = _ld(q_h, i * BQ, (i + 1) * BQ)
            L = (i + 1) * BQ
            chunks = []
            for a in range(0, L - BQ, CW):
                b = min(a + CW, L - BQ)
                chunks.append((a, b, _dot(q, _ld(k_s, a, b), NT)))
            sA = _dot(q, _ld(k_s, L - BQ, L - hb), NT)
            sA = jnp.where(c2 <= r2, sA, -1e30)
            chunks.append((L - BQ, L - hb, sA))
            sB = _dot(q[hb:], _ld(k_s, L - hb, L), NT)
            sB = jnp.where(c2[:hb] <= r2[:hb], sB, -1e30)
            m = None
            for (_, _, s) in chunks:
                mm = jnp.max(s, axis=1, keepdims=True)
                m = mm if m is None else jnp.maximum(m, mm)
            mB = jnp.maximum(m[hb:], jnp.max(sB, axis=1, keepdims=True))
            m = jnp.concatenate([m[:hb], mB], axis=0)
            return chunks, m, sB

        def pv(i, sc):
            chunks, m, sB = sc
            L = (i + 1) * BQ
            ctx = None
            l = None
            pB = jnp.exp2(sB - m[hb:])
            lB = jnp.sum(pB, axis=1, keepdims=True)
            cB = _dot(pB.astype(BF16), _ld(v_s, L - hb, L))
            for (a, b, s) in chunks:
                p = jnp.exp2(s - m)
                ll = jnp.sum(p, axis=1, keepdims=True)
                l = ll if l is None else l + ll
                d_ = _dot(p.astype(BF16), _ld(v_s, a, b))
                ctx = d_ if ctx is None else ctx + d_
            l = jnp.concatenate([l[:hb], l[hb:] + lB], axis=0)
            ctx = jnp.concatenate([ctx[:hb], ctx[hb:] + cB], axis=0)
            rr = gc_s[i * BQ:(i + 1) * BQ, :] / l
            return jnp.concatenate([ctx[:, :128] * rr, ctx[:, 128:] * rr], axis=1)

        def oproj(i):
            new = acc[:, i * BQ:(i + 1) * BQ] + _dot(woT, _ld(c_s, i * BQ, (i + 1) * BQ), NT)
            acc[:, i * BQ:(i + 1) * BQ] = new
            out_v[:, i * BQ:(i + 1) * BQ] = _cv(out_v, new)

            @pl.when(h == H - 1)
            def _():
                ocp[i].start()

        idx = list(reversed(range(nb)))
        sc = scores(idx[0])
        for n, i in enumerate(idx):
            cur = sc
            if n + 1 < nb:
                sc = scores(idx[n + 1])
            cr = BQ // (2 if c_s.dtype == U32 else 1)
            c_s[i * cr:(i + 1) * cr, :] = _cv(c_s, pv(i, cur))
            if n > 0:
                oproj(idx[n - 1])
        oproj(idx[-1])
        return carry

    with jax.named_scope('heads'):
        lax.fori_loop(0, H, head, 0)
    for cp in ocp:
        cp.wait()


@jax.jit
def pallas_gated_mix__compressed_kv_cla__linear_attn_block__prompt_kernel(
    A_x: jax.Array,
    A_c_kv: jax.Array,
    A_w_q: jax.Array,
    A_w_uk: jax.Array,
    A_w_uv: jax.Array,
    A_w_o: jax.Array,
    B_x: jax.Array,
    B_wqkv: jax.Array,
    B_wo: jax.Array,
    gate_w: jax.Array,
):
    U = ('ckv', 'k', 'v', 'c', 'x', 'xs', 'lhs')
    def B16(name, *shape):
        if name in U:
            return pltpu.VMEM((*shape[:-2], shape[-2] // 2, shape[-1]), U32)
        return pltpu.VMEM(shape, BF16)

    del B_x
    xT = jnp.swapaxes(A_x, 1, 2).reshape(M, S)
    ckv = A_c_kv.reshape(S, DC)
    woT = jnp.swapaxes(A_w_o, 1, 2)
    anyspec = pl.BlockSpec(memory_space=pl.ANY)
    outT = pl.pallas_call(
        _kernel,
        out_shape=jax.ShapeDtypeStruct((M, S), BF16),
        in_specs=[anyspec] * 9,
        out_specs=anyspec,
        scratch_shapes=[
            B16("x", M, S), B16("ckv", S, DC),
            pltpu.VMEM((H // 2, M, D), U32), pltpu.VMEM((H // 2, DC, D), U32), pltpu.VMEM((H // 2, DC, D), U32),
            B16("wo", H, M, D), pltpu.VMEM((M, 3 * M), BF16), pltpu.VMEM((M, M), BF16),
            pltpu.VMEM((M,), BF16),
            pltpu.VMEM((M, S), F32), pltpu.VMEM((8, S), F32),
            B16("xs", S, M),
            B16("q", H, S, D), B16("k", S, D), B16("v", S, D), B16("c", S, D),
            pltpu.VMEM((M, S), F32),
            pltpu.VMEM((S, 128), F32),
            B16("out", M, S),
            pltpu.VMEM((640, 128), F32), B16("lhs", 3 * M + 16, M), B16("w2", M, M),
            pltpu.VMEM((16, M), BF16),
            pltpu.SemaphoreType.DMA((30,)),
            pltpu.SemaphoreType.DMA((S // BQ,)),
            pltpu.SemaphoreType.DMA((S // CB,)),
        ],
        compiler_params=pltpu.CompilerParams(vmem_limit_bytes=100 * 1024 * 1024),
    )(xT, ckv, A_w_q, A_w_uk, A_w_uv, woT, B_wqkv, B_wo, gate_w)
    return jnp.swapaxes(outT.reshape(1, M, S), 1, 2)
```
